```python
import jax
import jax.numpy as jnp

def _softmax(x, axis=-1):
    return jax.nn.softmax(x, axis=axis)

def _gelu(x):
    return jax.nn.gelu(x, approximate=True)

def _silu(x):
    return jax.nn.silu(x)

def _sigmoid(x):
    return jax.nn.sigmoid(x)

def _layernorm(x, axis=-1, eps=1e-05):
    m = jnp.mean(x, axis=axis, keepdims=True)
    v = jnp.var(x, axis=axis, keepdims=True)
    return (x - m) / jnp.sqrt(v + eps)

def _scatter_add(tgt, idx, src, axis=0):
    return tgt.at[idx].add(src)

def _segment_sum(src, seg, n):
    return jax.ops.segment_sum(src, seg, n)

class _Rng:

    def __init__(self, key):
        self._k = key

    def _next(self):
        self._k, sub = jax.random.split(self._k)
        return sub

    def normal(self, shape):
        return jax.random.normal(self._next(), shape, dtype=jnp.bfloat16)

    def randint(self, lo, hi, shape):
        return jax.random.randint(self._next(), shape, lo, hi, dtype=jnp.int32)

    def uniform(self, shape, lo=0.0, hi=1.0):
        return jax.random.uniform(self._next(), shape, jnp.bfloat16, lo, hi)

    def permutation(self, n):
        return jax.random.permutation(self._next(), n)
kernel_name = 'adaLN_cond__memory_aug_recurrent_mem_tr__dense_activation_gelu__prompt'

def setup_inputs():
    _rng = _Rng(jax.random.key(int.from_bytes(__import__("os").urandom(4), "little")))
    _w = lambda a: (lambda t: t.astype(jnp.bfloat16) if jnp.issubdtype(t.dtype, jnp.floating) else t)(jnp.asarray(a))

    def _A_setup():
        B, S, Dm = (1, 2048, 1024)
        H, Dh = (32, 128)
        M, seg = (8, 32)
        seg = min(seg, S)
        S = S // seg * seg
        return {'x': _w((lambda *s: _rng.normal(s) * 0.05)(B, S, Dm)), 'mem0': _w((lambda *s: _rng.normal(s) * 0.05)(B, M, Dm)), 'Wq': _w((lambda *s: _rng.normal(s) * 0.05)(Dm, H, Dh) * Dm ** (-0.5)), 'Wk': _w((lambda *s: _rng.normal(s) * 0.05)(Dm, H, Dh) * Dm ** (-0.5)), 'Wv': _w((lambda *s: _rng.normal(s) * 0.05)(Dm, H, Dh) * Dm ** (-0.5)), 'Wo': _w((lambda *s: _rng.normal(s) * 0.05)(H, Dh, Dm) * (H * Dh) ** (-0.5)), 'seg_len': seg}
    _A_in = _A_setup()

    def _B_setup():
        B, S, D, F = (1, 2048, 1024, 3584)
        return {'x': _w((lambda *s: _rng.normal(s) * 0.05)(B, S, D)), 'w1': _w((lambda *s: _rng.normal(s) * 0.05)(D, F) * D ** (-0.5)), 'b1': _w((lambda *s: _rng.normal(s) * 0.05)(F) * 0.01), 'w2': _w((lambda *s: _rng.normal(s) * 0.05)(F, D) * F ** (-0.5)), 'b2': _w((lambda *s: _rng.normal(s) * 0.05)(D) * 0.01)}
    _B_in = _B_setup()
    return {'A_x': _A_in['x'], 'A_mem0': _A_in['mem0'], 'A_Wq': _A_in['Wq'], 'A_Wk': _A_in['Wk'], 'A_Wv': _A_in['Wv'], 'A_Wo': _A_in['Wo'], 'A_seg_len': _A_in['seg_len'], 'B_x': _B_in['x'], 'B_w1': _B_in['w1'], 'B_b1': _B_in['b1'], 'B_w2': _B_in['w2'], 'B_b2': _B_in['b2'], 'c': _w((lambda *s: _rng.normal(s) * 0.05)(1, 1024)), 'w_mod': _w((lambda *s: _rng.normal(s) * 0.05)(1024, 6 * 1024) * 1024 ** (-0.5))}

def reference(A_x, A_mem0, A_Wq, A_Wk, A_Wv, A_Wo, A_seg_len, B_x, B_w1, B_b1, B_w2, B_b2, c, w_mod):

    def _A_ref(x, mem0, Wq, Wk, Wv, Wo, seg_len):
        B, S, Dm = x.shape
        H, Dh = (Wq.shape[1], Wq.shape[2])
        M = mem0.shape[1]
        scale = Dh ** (-0.5)
        n_seg = S // seg_len
        L = M + seg_len
        idx = jnp.arange(L)
        mask = (idx[:, None] < M) | (idx[:, None] >= idx[None, :])
        mem = mem0
        outs = []
        for s in range(n_seg):
            xs = x[:, s * seg_len:(s + 1) * seg_len, :].copy()
            h = jnp.concatenate([mem, xs], axis=1)
            q = jnp.einsum('btd,dhe->bhte', h, Wq)
            k = jnp.einsum('btd,dhe->bhte', h, Wk)
            v = jnp.einsum('btd,dhe->bhte', h, Wv)
            scores = jnp.einsum('bhqe,bhke->bhqk', q, k) * scale
            scores = jnp.where(mask[None, None], scores, -1000000000.0)
            p = _softmax(scores, axis=-1)
            o = jnp.einsum('bhqk,bhke->bhqe', p, v)
            o = jnp.einsum('bhte,hed->btd', o, Wo)
            mem = o[:, :M, :].copy()
            outs.append(o[:, M:, :])
        return jnp.concatenate(outs, axis=1)

    def _B_ref(x, w1, b1, w2, b2):
        h = jnp.einsum('bsd,df->bsf', x, w1) + b1
        h = _gelu(h)
        return jnp.einsum('bsf,fd->bsd', h, w2) + b2
    x = A_x
    mod = (_silu(c) @ w_mod).reshape(c.shape[0], 6, 1, -1)
    sa, ca, ga, sb, cb, gb = (mod[:, 0].copy(), mod[:, 1].copy(), mod[:, 2].copy(), mod[:, 3].copy(), mod[:, 4].copy(), mod[:, 5].copy())
    h = _layernorm(x, axis=-1) * (1 + ca) + sa
    x = x + ga * _A_ref(h, A_mem0, A_Wq, A_Wk, A_Wv, A_Wo, A_seg_len)
    h = _layernorm(x, axis=-1) * (1 + cb) + sb
    x = x + gb * _B_ref(h, B_w1, B_b1, B_w2, B_b2)
    return x
```

```python
import functools

import jax
import jax.numpy as jnp
import numpy as np
import jax.experimental.pallas as pl
import jax.experimental.pallas.tpu as pltpu

F32 = jnp.float32
BF16 = jnp.bfloat16
U32 = jnp.uint32


def _dot(a, b):
    return jax.lax.dot_general(a, b, (((1,), (0,)), ((), ())), preferred_element_type=F32)


def _dot_nt(a, b):
    return jax.lax.dot_general(a, b, (((1,), (1,)), ((), ())), preferred_element_type=F32)


def _ln(x, eps=1e-5):
    m = jnp.mean(x, axis=-1, keepdims=True)
    xc = x - m
    v = jnp.mean(xc * xc, axis=-1, keepdims=True)
    return xc * jax.lax.rsqrt(v + eps)


def _rb(x):
    return x.astype(BF16).astype(F32)


def _kernel(x_hbm, mem0_ref, wq_hbm, wk_hbm, wv_hbm, wo_hbm, w1_hbm, b1_ref, w2_hbm, b2_ref,
            c_ref, wmod_hbm, out_hbm,
            xs, hs, wqkv, wo, w1s, w2s, wmod, stage, osc, x1s, obuf, mods,
            sem_x, sem_mod, sem_st, sem_wo, sem_w, sem_out,
            *, S, D, H, DH, M, SEG, FF, MB):
    NSEG = S // SEG
    L = M + SEG
    NP = H // 2
    scale = DH ** (-0.5)

    cp_mod = pltpu.make_async_copy(wmod_hbm, wmod, sem_mod)
    cp_mod.start()
    cp_x = pltpu.make_async_copy(x_hbm, xs, sem_x)
    cp_x.start()
    w_u32 = [r.bitcast(U32) for r in (wq_hbm, wk_hbm, wv_hbm)]

    def st_copy(m, j, slot):
        return pltpu.make_async_copy(w_u32[j].at[:, m, :], stage.at[slot, j], sem_st.at[slot, j])

    for j in range(3):
        st_copy(0, j, 0).start()
    for j in range(3):
        st_copy(1, j, 1).start()

    cp_mod.wait()
    cc = c_ref[...].astype(F32)
    sc = (cc * jax.nn.sigmoid(cc)).astype(BF16)
    mods[...] = _dot(sc, wmod[...])
    sa = mods[:, 0 * D:1 * D]
    ca1 = 1.0 + mods[:, 1 * D:2 * D]

    cp_x.wait()

    def ln_body(i, _):
        r = pl.multiple_of(i * 256, 256)
        xx = xs[pl.ds(r, 256), :].astype(F32)
        hs[pl.ds(r, 256), :] = _rb(_ln(xx) * ca1 + sa)
        return 0

    jax.lax.fori_loop(0, S // 256, ln_body, 0)

    def relayout(m, _):
        slot = m % 2
        for j in range(3):
            st_copy(m, j, slot).wait()
        for j in range(3):
            for r in range(D // 128):
                u = stage[slot, j, pl.ds(r * 128, 128), :]
                lo = pltpu.bitcast(u << 16, F32).astype(BF16)
                hi = pltpu.bitcast(u & U32(0xFFFF0000), F32).astype(BF16)
                wqkv[j, 2 * m, pl.ds(r * 64, 64), :] = pltpu.bitcast(lo, U32)
                wqkv[j, 2 * m + 1, pl.ds(r * 64, 64), :] = pltpu.bitcast(hi, U32)

        @pl.when(m + 2 < NP)
        def _():
            for j in range(3):
                st_copy(m + 2, j, slot).start()
        return 0

    jax.lax.fori_loop(0, NP, relayout, 0)
    cp_wo = pltpu.make_async_copy(wo_hbm.bitcast(U32), wo, sem_wo)
    cp_wo.start()
    cp_w1 = pltpu.make_async_copy(w1_hbm, w1s, sem_w.at[0])
    cp_w2 = pltpu.make_async_copy(w2_hbm, w2s, sem_w.at[1])
    cp_w1.start()
    cp_w2.start()
    cp_wo.wait()

    ga = mods[:, 2 * D:3 * D]
    row = jax.lax.broadcasted_iota(jnp.int32, (L, L), 0)
    col = jax.lax.broadcasted_iota(jnp.int32, (L, L), 1)
    mask = (row < M) | (row >= col)

    def step(s, mem):
        r = pl.multiple_of(s * SEG, SEG)
        hcat = jnp.concatenate([mem, hs[pl.ds(r, SEG), :]], axis=0)
        for h in range(H):
            q = _dot(hcat, pltpu.bitcast(wqkv[0, h], BF16))
            k = _dot(hcat, pltpu.bitcast(wqkv[1, h], BF16))
            v = _dot(hcat, pltpu.bitcast(wqkv[2, h], BF16))
            sc_ = _dot_nt(_rb(q), k.astype(BF16)) * scale
            sc_ = jnp.where(mask, sc_, -1e9)
            mx = jnp.max(sc_, axis=-1, keepdims=True)
            e = jnp.exp(sc_ - mx)
            p = e / jnp.sum(e, axis=-1, keepdims=True)
            o = _dot(_rb(p), v.astype(BF16))
            osc[:, h * DH:(h + 1) * DH] = _rb(o)
        out = _dot(osc[...], pltpu.bitcast(wo[...], BF16))
        out = _rb(out)
        x1s[pl.ds(r, SEG), :] = xs[pl.ds(r, SEG), :].astype(F32) + ga * out[M:]
        return out[:M]

    jax.lax.fori_loop(0, NSEG, step, mem0_ref[...].astype(F32))

    cp_w1.wait()
    cp_w2.wait()
    sb = mods[:, 3 * D:4 * D]
    cb1 = 1.0 + mods[:, 4 * D:5 * D]
    gb = mods[:, 5 * D:6 * D]
    b1 = b1_ref[...].astype(F32)
    b2 = b2_ref[...].astype(F32)
    NB = S // MB

    def out_copy(i, slot):
        return pltpu.make_async_copy(obuf.at[slot], out_hbm.at[pl.ds(i * MB, MB), :], sem_out.at[slot])

    def mlp(i, _):
        r = pl.multiple_of(i * MB, MB)
        slot = i % 2
        x1 = x1s[pl.ds(r, MB), :]
        h2 = (_ln(x1) * cb1 + sb).astype(BF16)
        a = _dot(h2, w1s[...]) + b1
        g = jax.nn.gelu(a, approximate=True).astype(BF16)
        y = _dot(g, w2s[...]) + b2

        @pl.when(i >= 2)
        def _():
            out_copy(i - 2, slot).wait()
        obuf[slot] = (x1 + gb * y).astype(BF16)
        out_copy(i, slot).start()
        return 0

    jax.lax.fori_loop(0, NB, mlp, 0)
    out_copy(NB - 2, (NB - 2) % 2).wait()
    out_copy(NB - 1, (NB - 1) % 2).wait()


@functools.partial(jax.jit, static_argnames=("A_seg_len",))
def pallas_adaLN_cond__memory_aug_recurrent_mem_tr__dense_activation_gelu__prompt_kernel(
    A_x, A_mem0, A_Wq, A_Wk, A_Wv, A_Wo, A_seg_len, B_x, B_w1, B_b1, B_w2, B_b2, c, w_mod,
):
    B, S, D = A_x.shape
    assert B == 1
    H, DH = A_Wq.shape[1], A_Wq.shape[2]
    M = A_mem0.shape[1]
    SEG = A_seg_len
    FF = B_w1.shape[1]
    MB = 256
    kern = functools.partial(_kernel, S=S, D=D, H=H, DH=DH, M=M, SEG=SEG, FF=FF, MB=MB)
    any_spec = pl.BlockSpec(memory_space=pl.ANY)
    vm = pl.BlockSpec(memory_space=pltpu.VMEM)
    out = pl.pallas_call(
        kern,
        out_shape=jax.ShapeDtypeStruct((S, D), BF16),
        in_specs=[any_spec, vm, any_spec, any_spec, any_spec, any_spec, any_spec, vm, any_spec, vm,
                  vm, any_spec],
        out_specs=any_spec,
        scratch_shapes=[
            pltpu.VMEM((S, D), BF16),
            pltpu.VMEM((S, D), F32),
            pltpu.VMEM((3, H, D // 2, DH), U32),
            pltpu.VMEM((H * DH // 2, D), U32),
            pltpu.VMEM((D, FF), BF16),
            pltpu.VMEM((FF, D), BF16),
            pltpu.VMEM((D, 6 * D), BF16),
            pltpu.VMEM((2, 3, D, DH), U32),
            pltpu.VMEM((M + SEG, H * DH), F32),
            pltpu.VMEM((S, D), F32),
            pltpu.VMEM((2, MB, D), BF16),
            pltpu.VMEM((1, 6 * D), F32),
            pltpu.SemaphoreType.DMA,
            pltpu.SemaphoreType.DMA,
            pltpu.SemaphoreType.DMA((2, 3)),
            pltpu.SemaphoreType.DMA,
            pltpu.SemaphoreType.DMA((2,)),
            pltpu.SemaphoreType.DMA((2,)),
        ],
        compiler_params=pltpu.CompilerParams(vmem_limit_bytes=120 * 1024 * 1024),
    )(A_x.reshape(S, D), A_mem0.reshape(M, D), A_Wq, A_Wk, A_Wv, A_Wo.reshape(H * DH, D),
      B_w1, B_b1.reshape(1, FF), B_w2, B_b2.reshape(1, D), c, w_mod)
    return out.reshape(B, S, D)
```

```python
import functools

import jax
import jax.numpy as jnp
import numpy as np
import jax.experimental.pallas as pl
import jax.experimental.pallas.tpu as pltpu

F32 = jnp.float32
BF16 = jnp.bfloat16
U32 = jnp.uint32


def _dot(a, b):
    return jax.lax.dot_general(a, b, (((1,), (0,)), ((), ())), preferred_element_type=F32)


def _dot_nt(a, b):
    return jax.lax.dot_general(a, b, (((1,), (1,)), ((), ())), preferred_element_type=F32)


def _ln(x, eps=1e-5):
    m = jnp.mean(x, axis=-1, keepdims=True)
    xc = x - m
    v = jnp.mean(xc * xc, axis=-1, keepdims=True)
    return xc * jax.lax.rsqrt(v + eps)


def _rb(x):
    return x.astype(BF16).astype(F32)


def _kernel(x_hbm, mem0_ref, wq_hbm, wk_hbm, wv_hbm, wo_hbm, w1_hbm, b1_ref, w2_hbm, b2_ref,
            c_ref, wmod_hbm, out_hbm,
            xs, hs, wqkv, wo, w1s, w2s, wmod, osc, hp, pre, obuf, mods,
            sem_x, sem_mod, sem_st, sem_wo, sem_w, sem_out,
            *, S, D, H, DH, M, SEG, FF, MB):
    NSEG = S // SEG
    L = M + SEG
    NP = H // 2
    scale = DH ** (-0.5)

    PRE = 8
    KEEP = SEG - PRE
    NPRE = NSEG * PRE

    cp_mod0 = pltpu.make_async_copy(wmod_hbm.at[:, :2 * D], wmod.at[:, :2 * D], sem_mod.at[0])
    cp_mod1 = pltpu.make_async_copy(wmod_hbm.at[:, 2 * D:], wmod.at[:, 2 * D:], sem_mod.at[1])
    cp_x = pltpu.make_async_copy(x_hbm, xs, sem_x)
    cp_wo = pltpu.make_async_copy(wo_hbm.bitcast(U32), wo, sem_wo)
    cp_w1 = pltpu.make_async_copy(w1_hbm, w1s, sem_w.at[0])
    cp_w2 = pltpu.make_async_copy(w2_hbm, w2s, sem_w.at[1])
    w_u32 = [r.bitcast(U32) for r in (wq_hbm, wk_hbm, wv_hbm)]

    def st_copy(m, j):
        return pltpu.make_async_copy(w_u32[j].at[:, m, :], wqkv.at[j, m].reshape(D, DH), sem_st.at[j * NP + m])

    def wt(j, m, par):
        return pltpu.bitcast(wqkv[j, m, :, par].reshape(D // 2, DH), BF16)

    cp_mod0.start()
    cp_x.start()
    for j in range(3):
        st_copy(0, j).start()

    cp_mod0.wait()
    for m0 in range(1, 3):
        for j in range(3):
            st_copy(m0, j).start()
    cc = c_ref[...].astype(F32)
    sc = (cc * jax.nn.sigmoid(cc)).astype(BF16)
    mods[:, :2 * D] = _dot(sc, wmod[:, :2 * D])
    sa = mods[:, 0 * D:1 * D]
    ca1 = 1.0 + mods[:, 1 * D:2 * D]

    cp_x.wait()
    for m0 in range(3, NP):
        for j in range(3):
            st_copy(m0, j).start()
    cp_wo.start()
    cp_mod1.start()
    cp_w1.start()
    cp_w2.start()
    LB = 256

    def ln_body(i, _):
        r = pl.multiple_of(i * LB, LB)
        xx = xs[pl.ds(r, LB), :].astype(F32)
        hh = _rb(_ln(xx) * ca1 + sa)
        hs[pl.ds(r, LB), :] = hh
        hp_ = hh.reshape(LB // SEG, SEG, D)[:, KEEP:, :].reshape(LB // SEG * PRE, D)
        hp[pl.ds(pl.multiple_of(i * (LB // SEG * PRE), LB // SEG * PRE), LB // SEG * PRE), :] = hp_.astype(BF16)
        return 0

    with jax.named_scope('ln'):
        jax.lax.fori_loop(0, S // LB, ln_body, 0)

    def relayout(m, j):
        for r in range(D // 128):
            u = wqkv[j, m, 8 * r:8 * r + 8].reshape(128, DH)
            lo = pltpu.bitcast(u << 16, F32).astype(BF16)
            hi = pltpu.bitcast(u & U32(0xFFFF0000), F32).astype(BF16)
            wqkv[j, m, 8 * r:8 * r + 8, 0] = pltpu.bitcast(lo, U32).reshape(8, 8, DH)
            wqkv[j, m, 8 * r:8 * r + 8, 1] = pltpu.bitcast(hi, U32).reshape(8, 8, DH)

    def pre_proj(m, j):
        for hh in range(2):
            y = _dot(hp[...], wt(j, m, hh))
            pre[j, 2 * m + hh] = _rb(y)

    for j in range(3):
        st_copy(0, j).wait()
        relayout(0, j)

    def pre_body(m, _):
        for j in range(3):
            st_copy(m + 1, j).wait()
        for j in range(3):
            relayout(m + 1, j)
            pre_proj(m, j)
        return 0

    with jax.named_scope('pre'):
        jax.lax.fori_loop(0, NP - 1, pre_body, 0)
        for j in range(3):
            pre_proj(NP - 1, j)
    with jax.named_scope('wowait'):
        cp_mod1.wait()
        mods[:, 2 * D:] = _dot(sc, wmod[:, 2 * D:])
        cp_wo.wait()

    ga = mods[:, 2 * D:3 * D]
    row = jax.lax.broadcasted_iota(jnp.int32, (L, L), 0)
    col = jax.lax.broadcasted_iota(jnp.int32, (L, L), 1)
    mask = (row < M) | (row >= col)

    def step(s, mem):
        r = pl.multiple_of(s * SEG, SEG)
        hcat = jnp.concatenate([mem, hs[pl.ds(r, KEEP), :]], axis=0).astype(BF16)
        rp = pl.multiple_of(s * PRE, PRE)
        st = {}

        def proj(j, h):
            y = _dot(hcat, wt(j, h // 2, h % 2))
            if j == 0:
                y = _rb(y)
            return jnp.concatenate([y, pre[j, h, pl.ds(rp, PRE), :]], axis=0)

        def scores(h):
            q, k = st.pop(("q", h)), st.pop(("k", h))
            sc_ = _dot_nt(q, k) * scale
            sc_ = jnp.where(mask, sc_, -1e9)
            mx = jnp.max(sc_, axis=-1, keepdims=True)
            e = jnp.exp(sc_ - mx)
            st["p", h] = _rb(e / jnp.sum(e, axis=-1, keepdims=True))

        def pv(h):
            o = _dot(st.pop(("p", h)), st.pop(("v", h)))
            osc[:, h * DH:(h + 1) * DH] = _rb(o)

        def wo_part(h0, h1):
            y = _dot(osc[:, h0 * DH:h1 * DH],
                     pltpu.bitcast(wo[h0 * DH // 2:h1 * DH // 2, :], BF16))
            st["acc"] = y if "acc" not in st else st["acc"] + y

        G = 4
        NG = H // G
        for g in range(NG):
            for i in range(g * G, g * G + G):
                st["q", i] = proj(0, i)
            if g >= 1:
                for i in range(g * G - G, g * G):
                    scores(i)
            for i in range(g * G, g * G + G):
                st["k", i] = proj(1, i).astype(BF16)
            if g >= 1:
                for i in range(g * G - G, g * G):
                    pv(i)
            for i in range(g * G, g * G + G):
                st["v", i] = proj(2, i).astype(BF16)
        wo_part(0, 4)
        for i in range(H - G, H):
            scores(i)
        wo_part(4, 16)
        for i in range(H - G, H):
            pv(i)
        wo_part(16, 28)
        wo_part(28, 32)
        out = st.pop("acc")
        out = _rb(out)
        hs[pl.ds(r, SEG), :] = xs[pl.ds(r, SEG), :].astype(F32) + ga * out[M:]
        return out[:M]

    with jax.named_scope('chain'):
        jax.lax.fori_loop(0, NSEG, step, mem0_ref[...].astype(F32))

    cp_w1.wait()
    cp_w2.wait()
    sb = mods[:, 3 * D:4 * D]
    cb1 = 1.0 + mods[:, 4 * D:5 * D]
    gb = mods[:, 5 * D:6 * D]
    b1 = b1_ref[...].astype(F32)
    b2 = b2_ref[...].astype(F32)
    NB = S // MB

    def out_copy(i, slot):
        return pltpu.make_async_copy(obuf.at[slot], out_hbm.at[pl.ds(i * MB, MB), :], sem_out.at[slot])

    def mlp(i, _):
        r = pl.multiple_of(i * MB, MB)
        slot = i % 2
        x1 = hs[pl.ds(r, MB), :]
        h2 = (_ln(x1) * cb1 + sb).astype(BF16)
        a = _dot(h2, w1s[...]) + b1
        g = jax.nn.gelu(a, approximate=True).astype(BF16)
        y = _dot(g, w2s[...]) + b2

        @pl.when(i >= 2)
        def _():
            out_copy(i - 2, slot).wait()
        obuf[slot] = (x1 + gb * y).astype(BF16)
        out_copy(i, slot).start()
        return 0

    with jax.named_scope('mlp'):
        jax.lax.fori_loop(0, NB, mlp, 0)
    out_copy(NB - 2, (NB - 2) % 2).wait()
    out_copy(NB - 1, (NB - 1) % 2).wait()


@functools.partial(jax.jit, static_argnames=("A_seg_len",))
def pallas_adaLN_cond__memory_aug_recurrent_mem_tr__dense_activation_gelu__prompt_kernel(
    A_x, A_mem0, A_Wq, A_Wk, A_Wv, A_Wo, A_seg_len, B_x, B_w1, B_b1, B_w2, B_b2, c, w_mod,
):
    B, S, D = A_x.shape
    assert B == 1
    H, DH = A_Wq.shape[1], A_Wq.shape[2]
    M = A_mem0.shape[1]
    SEG = A_seg_len
    FF = B_w1.shape[1]
    MB = 256
    kern = functools.partial(_kernel, S=S, D=D, H=H, DH=DH, M=M, SEG=SEG, FF=FF, MB=MB)
    any_spec = pl.BlockSpec(memory_space=pl.ANY)
    vm = pl.BlockSpec(memory_space=pltpu.VMEM)
    out = pl.pallas_call(
        kern,
        out_shape=jax.ShapeDtypeStruct((S, D), BF16),
        in_specs=[any_spec, vm, any_spec, any_spec, any_spec, any_spec, any_spec, vm, any_spec, vm,
                  vm, any_spec],
        out_specs=any_spec,
        scratch_shapes=[
            pltpu.VMEM((S, D), BF16),
            pltpu.VMEM((S, D), F32),
            pltpu.VMEM((3, H // 2, D // 16, 2, 8, DH), U32),
            pltpu.VMEM((H * DH // 2, D), U32),
            pltpu.VMEM((D, FF), BF16),
            pltpu.VMEM((FF, D), BF16),
            pltpu.VMEM((D, 6 * D), BF16),
            pltpu.VMEM((M + SEG, H * DH), F32),
            pltpu.VMEM((S // SEG * 8, D), BF16),
            pltpu.VMEM((3, H, S // SEG * 8, DH), F32),
            pltpu.VMEM((2, MB, D), BF16),
            pltpu.VMEM((1, 6 * D), F32),
            pltpu.SemaphoreType.DMA,
            pltpu.SemaphoreType.DMA((2,)),
            pltpu.SemaphoreType.DMA((3 * H // 2,)),
            pltpu.SemaphoreType.DMA,
            pltpu.SemaphoreType.DMA((2,)),
            pltpu.SemaphoreType.DMA((2,)),
        ],
        compiler_params=pltpu.CompilerParams(vmem_limit_bytes=120 * 1024 * 1024),
    )(A_x.reshape(S, D), A_mem0.reshape(M, D), A_Wq, A_Wk, A_Wv, A_Wo.reshape(H * DH, D),
      B_w1, B_b1.reshape(1, FF), B_w2, B_b2.reshape(1, D), c, w_mod)
    return out.reshape(B, S, D)
```

```python
import functools

import jax
import jax.numpy as jnp
import numpy as np
import jax.experimental.pallas as pl
import jax.experimental.pallas.tpu as pltpu

F32 = jnp.float32
BF16 = jnp.bfloat16
U32 = jnp.uint32


def _dot(a, b):
    return jax.lax.dot_general(a, b, (((1,), (0,)), ((), ())), preferred_element_type=F32)


def _dot_nt(a, b):
    return jax.lax.dot_general(a, b, (((1,), (1,)), ((), ())), preferred_element_type=F32)


def _ln(x, eps=1e-5):
    m = jnp.mean(x, axis=-1, keepdims=True)
    xc = x - m
    v = jnp.mean(xc * xc, axis=-1, keepdims=True)
    return xc * jax.lax.rsqrt(v + eps)


def _rb(x):
    return x.astype(BF16).astype(F32)


def _kernel(x_hbm, mem0_ref, wq_hbm, wk_hbm, wv_hbm, wo_hbm, w1_hbm, b1_ref, w2_hbm, b2_ref,
            c_ref, wmod_hbm, out_hbm,
            xs, xp, hs, wqkv, wo, w1s, w2s, wmod, osc, hp, pre, obuf, mods,
            sem_x, sem_mod, sem_st, sem_wo, sem_w, sem_out,
            *, S, D, H, DH, M, SEG, FF, MB):
    NSEG = S // SEG
    L = M + SEG
    NP = H // 2
    scale = DH ** (-0.5)

    PRE = 8
    KEEP = SEG - PRE
    NPRE = NSEG * PRE

    cp_mod0 = pltpu.make_async_copy(wmod_hbm.at[:, :2 * D], wmod.at[:, :2 * D], sem_mod.at[0])
    cp_mod1 = pltpu.make_async_copy(wmod_hbm.at[:, 2 * D:], wmod.at[:, 2 * D:], sem_mod.at[1])
    cp_x = pltpu.make_async_copy(x_hbm, xs, sem_x.at[0])
    cp_xp = pltpu.make_async_copy(x_hbm.at[:, KEEP:, :], xp, sem_x.at[1])
    cp_wo = pltpu.make_async_copy(wo_hbm.bitcast(U32), wo, sem_wo)
    cp_w1 = pltpu.make_async_copy(w1_hbm, w1s, sem_w.at[0])
    cp_w2 = pltpu.make_async_copy(w2_hbm, w2s, sem_w.at[1])
    w_u32 = [r.bitcast(U32) for r in (wq_hbm, wk_hbm, wv_hbm)]

    def st_copy(m, j):
        return pltpu.make_async_copy(w_u32[j].at[:, m, :], wqkv.at[j, m].reshape(D, DH), sem_st.at[j * NP + m])

    def wt(j, m, par):
        return pltpu.bitcast(wqkv[j, m, :, par].reshape(D // 2, DH), BF16)

    cp_mod0.start()
    cp_xp.start()
    for j in range(3):
        st_copy(0, j).start()

    cp_mod0.wait()
    for m0 in range(1, 3):
        for j in range(3):
            st_copy(m0, j).start()
    cc = c_ref[...].astype(F32)
    sc = (cc * jax.nn.sigmoid(cc)).astype(BF16)
    mods[:, :2 * D] = _dot(sc, wmod[:, :2 * D])
    sa = mods[:, 0 * D:1 * D]
    ca1 = 1.0 + mods[:, 1 * D:2 * D]

    cp_xp.wait()
    for m0 in range(3, NP):
        for j in range(3):
            st_copy(m0, j).start()
    cp_x.start()
    cp_wo.start()
    cp_mod1.start()
    with jax.named_scope('ln'):
        for i in range(NSEG // 16):
            xx = xp[16 * i:16 * i + 16].astype(F32).reshape(16 * PRE, D)
            hh = (_ln(xx) * ca1 + sa).astype(BF16)
            hp[8 * PRE * i:8 * PRE * (i + 1), :] = pltpu.bitcast(hh, U32)

    def ln_seg(s_):
        xx = xs[s_, :KEEP, :].astype(F32)
        hs[s_, :KEEP, :] = _rb(_ln(xx) * ca1 + sa)

    def relayout(m, j):
        for r in range(D // 128):
            u = wqkv[j, m, 8 * r:8 * r + 8].reshape(128, DH)
            lo = pltpu.bitcast(u << 16, F32).astype(BF16)
            hi = pltpu.bitcast(u & U32(0xFFFF0000), F32).astype(BF16)
            wqkv[j, m, 8 * r:8 * r + 8, 0] = pltpu.bitcast(lo, U32).reshape(8, 8, DH)
            wqkv[j, m, 8 * r:8 * r + 8, 1] = pltpu.bitcast(hi, U32).reshape(8, 8, DH)

    def pre_proj(m, j):
        for hh in range(2):
            y = _dot(pltpu.bitcast(hp[...], BF16), wt(j, m, hh))
            pre[j, 2 * m + hh] = _rb(y)

    for j in range(3):
        st_copy(0, j).wait()
        relayout(0, j)

    def pre_body(m, _):
        for j in range(3):
            st_copy(m + 1, j).wait()
        for j in range(3):
            relayout(m + 1, j)
            pre_proj(m, j)
        return 0

    with jax.named_scope('pre'):
        jax.lax.fori_loop(0, NP - 1, pre_body, 0)
        for j in range(3):
            pre_proj(NP - 1, j)
    with jax.named_scope('wowait'):
        cp_mod1.wait()
        mods[:, 2 * D:] = _dot(sc, wmod[:, 2 * D:])
        cp_wo.wait()
        cp_w1.start()
        cp_w2.start()
        cp_x.wait()
        ln_seg(0)

    ga = mods[:, 2 * D:3 * D]
    row = jax.lax.broadcasted_iota(jnp.int32, (L, L), 0)
    col = jax.lax.broadcasted_iota(jnp.int32, (L, L), 1)
    mask = (row < M) | (row >= col)

    def step(s, mem):
        r = pl.multiple_of(s * SEG, SEG)
        hcat = jnp.concatenate([mem, hs[s, :KEEP, :]], axis=0).astype(BF16)
        rp = pl.multiple_of(s * PRE, PRE)
        st = {}

        def proj(j, h):
            y = _dot(hcat, wt(j, h // 2, h % 2))
            if j == 0:
                y = _rb(y)
            return jnp.concatenate([y, pre[j, h, pl.ds(rp, PRE), :]], axis=0)

        def scores(h):
            q, k = st.pop(("q", h)), st.pop(("k", h))
            st["s", h] = _dot_nt(q, k)

        def softmax(h):
            sc_ = st.pop(("s", h)) * scale
            sc_ = jnp.where(mask, sc_, -1e9)
            mx = jnp.max(sc_, axis=-1, keepdims=True)
            e = jnp.exp(sc_ - mx)
            st["p", h] = _rb(e / jnp.sum(e, axis=-1, keepdims=True))

        def pv(h):
            o = _dot(st.pop(("p", h)), st.pop(("v", h)))
            osc[:, h * DH:(h + 1) * DH] = _rb(o)

        def wo_part(h0, h1):
            y = _dot(osc[:, h0 * DH:h1 * DH],
                     pltpu.bitcast(wo[h0 * DH // 2:h1 * DH // 2, :], BF16))
            st["acc"] = y if "acc" not in st else st["acc"] + y

        G = 4
        NG = H // G
        ORDER = [('q', 0, 4), ('s', 0, 4), ('k', 0, 2), ('m', 0, 4), ('k', 2, 4), ('v', 0, 2), ('p', 0, 4), ('v', 2, 4)]

        def do(op, g, lo=0, hi=None):
            for i in range(g * G + lo, g * G + (G if hi is None else hi)):
                if op in "qkv":
                    y = proj("qkv".index(op), i)
                    st[op, i] = y if op == "q" else y.astype(BF16)
                else:
                    dict(s=scores, m=softmax, p=pv)[op](i)

        for g in range(NG):
            for op, lo, hi in ORDER:
                if op in "qkv":
                    do(op, g, lo, hi)
                elif g >= 1:
                    do(op, g - 1, lo, hi)
        ln_seg(jnp.minimum(s + 1, NSEG - 1))
        wo_part(0, 4)
        do("s", NG - 1)
        wo_part(4, 8)
        do("m", NG - 1)
        wo_part(8, 16)
        do("p", NG - 1)
        wo_part(16, 32 - G)
        wo_part(32 - G, 32)
        out = st.pop("acc")
        out = _rb(out)
        hs[s] = xs[s].astype(F32) + ga * out[M:]
        return out[:M]

    with jax.named_scope('chain'):
        jax.lax.fori_loop(0, NSEG, step, mem0_ref[...].astype(F32))

    cp_w1.wait()
    cp_w2.wait()
    sb = mods[:, 3 * D:4 * D]
    cb1 = 1.0 + mods[:, 4 * D:5 * D]
    gb = mods[:, 5 * D:6 * D]
    b1 = b1_ref[...].astype(F32)
    b2 = b2_ref[...].astype(F32)
    NB = S // MB

    def out_copy(i, slot):
        return pltpu.make_async_copy(obuf.at[slot], out_hbm.at[pl.ds(i * MB, MB), :], sem_out.at[slot])

    def mlp(i, _):
        r = pl.multiple_of(i * MB, MB)
        slot = i % 2
        x1 = hs[pl.ds(pl.multiple_of(i * (MB // SEG), MB // SEG), MB // SEG)].reshape(MB, D)
        h2 = (_ln(x1) * cb1 + sb).astype(BF16)
        a = _dot(h2, w1s[...]) + b1
        g = jax.nn.gelu(a, approximate=True).astype(BF16)
        y = _dot(g, w2s[...]) + b2

        @pl.when(i >= 2)
        def _():
            out_copy(i - 2, slot).wait()
        obuf[slot] = (x1 + gb * y).astype(BF16)
        out_copy(i, slot).start()
        return 0

    with jax.named_scope('mlp'):
        jax.lax.fori_loop(0, NB, mlp, 0)
    out_copy(NB - 2, (NB - 2) % 2).wait()
    out_copy(NB - 1, (NB - 1) % 2).wait()


@functools.partial(jax.jit, static_argnames=("A_seg_len",))
def pallas_adaLN_cond__memory_aug_recurrent_mem_tr__dense_activation_gelu__prompt_kernel(
    A_x, A_mem0, A_Wq, A_Wk, A_Wv, A_Wo, A_seg_len, B_x, B_w1, B_b1, B_w2, B_b2, c, w_mod,
):
    B, S, D = A_x.shape
    assert B == 1
    H, DH = A_Wq.shape[1], A_Wq.shape[2]
    M = A_mem0.shape[1]
    SEG = A_seg_len
    FF = B_w1.shape[1]
    MB = 256
    kern = functools.partial(_kernel, S=S, D=D, H=H, DH=DH, M=M, SEG=SEG, FF=FF, MB=MB)
    any_spec = pl.BlockSpec(memory_space=pl.ANY)
    vm = pl.BlockSpec(memory_space=pltpu.VMEM)
    out = pl.pallas_call(
        kern,
        out_shape=jax.ShapeDtypeStruct((S, D), BF16),
        in_specs=[any_spec, vm, any_spec, any_spec, any_spec, any_spec, any_spec, vm, any_spec, vm,
                  vm, any_spec],
        out_specs=any_spec,
        scratch_shapes=[
            pltpu.VMEM((S // SEG, SEG, D), BF16),
            pltpu.VMEM((S // SEG, 8, D), BF16),
            pltpu.VMEM((S // SEG, SEG, D), F32),
            pltpu.VMEM((3, H // 2, D // 16, 2, 8, DH), U32),
            pltpu.VMEM((H * DH // 2, D), U32),
            pltpu.VMEM((D, FF), BF16),
            pltpu.VMEM((FF, D), BF16),
            pltpu.VMEM((D, 6 * D), BF16),
            pltpu.VMEM((M + SEG, H * DH), F32),
            pltpu.VMEM((S // SEG * 4, D), U32),
            pltpu.VMEM((3, H, S // SEG * 8, DH), F32),
            pltpu.VMEM((2, MB, D), BF16),
            pltpu.VMEM((1, 6 * D), F32),
            pltpu.SemaphoreType.DMA((2,)),
            pltpu.SemaphoreType.DMA((2,)),
            pltpu.SemaphoreType.DMA((3 * H // 2,)),
            pltpu.SemaphoreType.DMA,
            pltpu.SemaphoreType.DMA((2,)),
            pltpu.SemaphoreType.DMA((2,)),
        ],
        compiler_params=pltpu.CompilerParams(vmem_limit_bytes=120 * 1024 * 1024),
    )(A_x.reshape(S // SEG, SEG, D), A_mem0.reshape(M, D), A_Wq, A_Wk, A_Wv, A_Wo.reshape(H * DH, D),
      B_w1, B_b1.reshape(1, FF), B_w2, B_b2.reshape(1, D), c, w_mod)
    return out.reshape(B, S, D)
```
